```python
import jax
import jax.numpy as jnp

def _softmax(x, axis=-1):
    return jax.nn.softmax(x, axis=axis)
def _gelu(x):
    return jax.nn.gelu(x, approximate=True)
def _silu(x):
    return jax.nn.silu(x)
def _sigmoid(x):
    return jax.nn.sigmoid(x)
def _layernorm(x, axis=-1, eps=1e-5):
    m = jnp.mean(x, axis=axis, keepdims=True)
    v = jnp.var(x, axis=axis, keepdims=True)
    return (x - m) / jnp.sqrt(v + eps)
def _scatter_add(tgt, idx, src, axis=0):
    return tgt.at[idx].add(src)
def _segment_sum(src, seg, n):
    return jax.ops.segment_sum(src, seg, n)
class _Rng:
    def __init__(self, key):
        self._k = key
    def _next(self):
        self._k, sub = jax.random.split(self._k)
        return sub
    def normal(self, shape):
        return jax.random.normal(self._next(), shape, dtype=jnp.bfloat16)
    def randint(self, lo, hi, shape):
        return jax.random.randint(self._next(), shape, lo, hi, dtype=jnp.int32)
    def uniform(self, shape, lo=0.0, hi=1.0):
        return jax.random.uniform(self._next(), shape, jnp.bfloat16, lo, hi)
    def permutation(self, n):
        return jax.random.permutation(self._next(), n)


kernel_name = 'sequential_preLN__sliding_block__glu_gated_glu__prompt'

def _fwd_setup_inputs():
    _rng = _Rng(jax.random.key(int.from_bytes(__import__("os").urandom(4), "little")))
    _w = (lambda a: (lambda t: t.astype(jnp.bfloat16) if jnp.issubdtype(t.dtype, jnp.floating) else t)(jnp.asarray(a)))
    def _A_setup():
        B, S, D = 1, 2048, 512
        return {
            "x": _w((lambda *s: _rng.normal(s) * 0.05)(B, S, D)),
            "wqkv": _w((lambda *s: _rng.normal(s) * 0.05)(D, 3 * D)),
            "wo": _w((lambda *s: _rng.normal(s) * 0.05)(D, D)),
        }
    _A_in = _A_setup()

    def _B_setup():
        B, S, D, F = 1, 2048, 512, 1376
        return {
            "x": _w((lambda *s: _rng.normal(s) * 0.05)(B, S, D)),
            "w_gate": _w((lambda *s: _rng.normal(s) * 0.05)(D, F)),
            "w_up": _w((lambda *s: _rng.normal(s) * 0.05)(D, F)),
            "w_down": _w((lambda *s: _rng.normal(s) * 0.05)(F, D)),
        }
    _B_in = _B_setup()

    return {
        "A_x": _A_in["x"],
        "A_wqkv": _A_in["wqkv"],
        "A_wo": _A_in["wo"],
        "B_x": _B_in["x"],
        "B_w_gate": _B_in["w_gate"],
        "B_w_up": _B_in["w_up"],
        "B_w_down": _B_in["w_down"],
    }

def _fwd_reference(A_x, A_wqkv, A_wo, B_x, B_w_gate, B_w_up, B_w_down):
    def _A_ref(x, wqkv, wo):
        B, S, D = x.shape
        H = 32; Dh = D // H; W = 256
        qkv = (lambda x, *d: x.transpose(*d))((x @ wqkv).reshape(B, S, 3, H, Dh), 2, 0, 3, 1, 4)
        q, k, v = qkv[0], qkv[1], qkv[2]
        scores = jnp.einsum("bhqd,bhkd->bhqk", q, k) * (Dh ** -0.5)
        idx = jnp.arange(S)
        mask = (idx[:, None] - idx[None, :] >= 0) & (idx[:, None] - idx[None, :] < W)
        scores = jnp.where(mask[None, None], scores, -1e9)
        p = _softmax(scores, axis=-1)
        o = jnp.einsum("bhqk,bhkd->bhqd", p, v)
        return (lambda x, *d: x.transpose(*d))(o, 0, 2, 1, 3).reshape(B, S, D) @ wo

    def _B_ref(x, w_gate, w_up, w_down):
        g = jnp.einsum("bsd,df->bsf", x, w_gate)
        u = jnp.einsum("bsd,df->bsf", x, w_up)
        h = _sigmoid(g) * u
        return jnp.einsum("bsf,fd->bsd", h, w_down)

    x = A_x
    h = x + _A_ref(_layernorm(x, axis=-1), A_wqkv, A_wo)
    h2 = h + _B_ref(_layernorm(h, axis=-1), B_w_gate, B_w_up, B_w_down)
    return h2


def setup_inputs():
    _inp = _fwd_setup_inputs()
    _gk = jax.random.fold_in(jax.random.key(int.from_bytes(__import__("os").urandom(4), "little")), 2**31 - 1)
    _shapes = [[1, 2048, 512]]
    _dtypes = ['bfloat16']
    _gks = jax.random.split(_gk, len(_shapes))
    _gs = [jax.random.normal(k, s, dtype=jnp.dtype(d)) * 0.05 for k, s, d in zip(_gks, _shapes, _dtypes)]
    _inp["grad_out"] = _gs[0]
    return _inp

def reference(A_x, A_wqkv, A_wo, B_w_gate, B_w_up, B_w_down, B_x, grad_out):
    _const = dict(B_x=B_x)
    def _f(*_d):
        return _fwd_reference(**{'A_x': _d[0], 'A_wqkv': _d[1], 'A_wo': _d[2], 'B_w_gate': _d[3], 'B_w_up': _d[4], 'B_w_down': _d[5], **_const})
    _out, _vjp = jax.vjp(_f, A_x, A_wqkv, A_wo, B_w_gate, B_w_up, B_w_down)
    _grads = _vjp(grad_out)
    _out0 = jnp.asarray(_out)
    return (_out0, *[jnp.asarray(_g) for _g in _grads])
```

```python
import functools

import jax
import jax.numpy as jnp
from jax import lax
import jax.experimental.pallas as pl
import jax.experimental.pallas.tpu as pltpu

F32 = jnp.float32
BF16 = jnp.bfloat16

H = 32
DH = 16
W = 256
EPS = 1e-5
NEG = -1e9
BIG = 3e38

QB = 128
KW = QB + W
HG = 128 // DH
T = 512
LOG2E = 1.4426950408889634
LN2 = 0.6931471805599453
VR = 2 * DH
NQB = T // QB


def _dot(a, b):
    return jnp.dot(a, b, preferred_element_type=F32)


def _dot_nt(a, b):
    return lax.dot_general(a, b, (((1,), (1,)), ((), ())), preferred_element_type=F32)


def _dot_tn(a, b):
    return lax.dot_general(a, b, (((0,), (0,)), ((), ())), preferred_element_type=F32)


def _ln_stats(x):
    mu = jnp.mean(x, axis=-1, keepdims=True)
    xc = x - mu
    var = jnp.mean(xc * xc, axis=-1, keepdims=True)
    rstd = lax.rsqrt(var + EPS)
    return xc * rstd, rstd


def _ln_bwd(dy, y, rstd):
    return rstd * (
        dy
        - jnp.mean(dy, axis=-1, keepdims=True)
        - y * jnp.mean(dy * y, axis=-1, keepdims=True)
    )


def _keep_head(at, h):
    row_head = lax.broadcasted_iota(jnp.int32, at.shape, 0) // DH
    return jnp.where(row_head == h, at, jnp.zeros_like(at))


def _kernel(
    x_ref, go_ref, wqkv_hbm, wo_hbm, wgt_hbm, wut_hbm, wd_hbm,
    out_ref, dx_ref, dwqkv_hbm, dwo_hbm, dwgt_hbm, dwut_hbm, dwd_hbm,
    wqkv_ref, wo_ref, wgt_ref, wut_ref, wd_ref, sem_in,
    s_wqkv, s_wo, s_wgt, s_wut, s_wd, sem_out,
    qtbuf, kbuf, vbuf, ktbuf, vtbuf, pbuf, dsbuf, sbuf, mbuf, dbuf, dosb, capbuf, linv,
    otbuf, dotbuf, dqtbuf, dk_acc, dv_acc,
    dhbuf, y1buf, r1buf,
    a_wqkv, a_wo, a_wg, a_wu, a_wdt,
    y2buf, y2tbuf, dytbuf, yacc, dy2acc,
    *, n_blocks, d_model, d_ff,
):
    i = pl.program_id(0)
    n_grp = d_model // 128
    n_fc = pl.cdiv(d_ff, 128)
    slot = i % 2

    w_in = [
        pltpu.make_async_copy(src, dst, sem_in.at[k])
        for k, (src, dst) in enumerate(
            [(wqkv_hbm, wqkv_ref), (wo_hbm, wo_ref), (wgt_hbm, wgt_ref.at[0:d_ff]),
             (wut_hbm, wut_ref.at[0:d_ff]), (wd_hbm, wd_ref.at[0:d_ff])]
        )
    ]
    w_out = [
        pltpu.make_async_copy(src, dst, sem_out.at[k])
        for k, (src, dst) in enumerate(
            [(s_wqkv, dwqkv_hbm), (s_wo, dwo_hbm), (s_wgt, dwgt_hbm),
             (s_wut, dwut_hbm), (s_wd, dwd_hbm)]
        )
    ]

    @pl.when(i == 0)
    def _init():
        with jax.named_scope('init'):
            for c in w_in:
                c.start()
            tail = vtbuf.shape[:2] + (VR - DH, vtbuf.shape[3])
            ones_row = lax.broadcasted_iota(jnp.int32, tail, 2) == 0
            vtbuf[:, :, DH:, :] = ones_row.astype(BF16)
            a_wqkv[...] = jnp.zeros_like(a_wqkv)
            a_wo[...] = jnp.zeros_like(a_wo)
            a_wg[...] = jnp.zeros_like(a_wg)
            a_wu[...] = jnp.zeros_like(a_wu)
            a_wdt[...] = jnp.zeros_like(a_wdt)
            if n_fc * 128 > d_ff:
                pad = jnp.zeros((n_fc * 128 - d_ff, d_model), BF16)
                wgt_ref[d_ff:, :] = pad
                wut_ref[d_ff:, :] = pad
                wd_ref[d_ff:, :] = pad
            w_in[0].wait()

    @pl.when(i < n_blocks)
    def _forward_and_local_backward():
        r0 = pl.multiple_of(i * T, T)
        with jax.named_scope('qkv'):
            x = x_ref[...].astype(F32)
            y1, rstd1 = _ln_stats(x)
            y1buf[slot] = y1
            r1buf[slot] = rstd1
            qkv = _dot(y1.astype(BF16), wqkv_ref[...])
            kv0 = pl.multiple_of(r0 + W, 128)
            dytbuf[...] = go_ref[...].astype(F32).T.astype(BF16)
            dy2acc[...] = jnp.zeros_like(dy2acc)
            for g in range(n_grp):
                lo = g * 128
                qtbuf[g] = (qkv[:, lo:lo + 128] * (DH ** -0.5 * LOG2E)).T.astype(BF16)
                kg = qkv[:, d_model + lo:d_model + lo + 128]
                vg = qkv[:, 2 * d_model + lo:2 * d_model + lo + 128]
                kbuf[g, pl.ds(kv0, T), :] = kg.astype(BF16)
                vbuf[g, pl.ds(kv0, T), :] = vg.astype(BF16)
                ktbuf[g, :, pl.ds(kv0, T)] = kg.T.astype(BF16)
                vgt = vg.T.astype(BF16)
                for hh in range(HG):
                    vtbuf[g, hh, 0:DH, pl.ds(kv0, T)] = vgt[hh * DH:(hh + 1) * DH]

            for qb in range(NQB):
                q0 = r0 + qb * QB
                kpos = q0 - W + lax.broadcasted_iota(jnp.int32, (KW, QB), 0)
                qpos = q0 + lax.broadcasted_iota(jnp.int32, (KW, QB), 1)
                valid = (kpos >= 0) & (kpos <= qpos) & (qpos - kpos < W)
                capbuf[qb] = jnp.where(valid, BIG, NEG)

        def head_stack_t(at):
            return jnp.concatenate([_keep_head(at, h) for h in range(HG)], axis=1)

        def nkt_of(first):
            return lambda qb: min(qb + 1, KW // 128) if first else KW // 128

        def scores(qb, g, nkt):
            n = nkt(qb) * 128
            ks = KW - n
            q0 = pl.multiple_of(r0 + qb * QB + ks, QB)
            qt = qtbuf[g, :, qb * QB:(qb + 1) * QB]
            s = _dot(kbuf[g, pl.ds(q0, n), :], head_stack_t(qt))
            for h in range(HG):
                tiles = []
                for kt in range(ks // 128, KW // 128):
                    st = s[kt * 128 - ks:(kt + 1) * 128 - ks, h * QB:(h + 1) * QB]
                    if kt in (0, KW // 128 - 1):
                        st = jnp.minimum(st, capbuf[qb, kt * 128:(kt + 1) * 128, :])
                    tiles.append(st)
                sh = jnp.concatenate(tiles, axis=0) if len(tiles) > 1 else tiles[0]
                sbuf[qb, 0:n, h * QB:(h + 1) * QB] = sh
                mbuf[qb, h] = jnp.max(sh, axis=0, keepdims=True)

        def softmax_pv(qb, g, nkt):
            n = nkt(qb) * 128
            q0 = pl.multiple_of(r0 + qb * QB + KW - n, QB)
            for h in range(HG):
                p = jnp.exp2(sbuf[qb, 0:n, h * QB:(h + 1) * QB] - mbuf[qb, h])
                pbuf[qb, g, h, 0:n, :] = p.astype(BF16)
                ot = _dot(vtbuf[g, h, :, pl.ds(q0, n)], pbuf[qb, g, h, 0:n, :])
                li = 1.0 / ot[DH:DH + 1, :]
                linv[qb, g, h] = li
                otbuf[g, h * DH:(h + 1) * DH, qb * QB:(qb + 1) * QB] = ot[0:DH, :] * li

        def attention_fwd(first):
            nkt = nkt_of(first)

            def body(g, carry):
                for qb in range(NQB):
                    if qb + 1 < NQB:
                        scores(qb + 1, g, nkt)
                    else:
                        scores(0, jnp.minimum(g + 1, n_grp - 1), nkt)
                    softmax_pv(qb, g, nkt)
                return carry

            scores(0, 0, nkt)
            lax.fori_loop(0, n_grp, body, 0)

        with jax.named_scope('attn_fwd'):
            pl.when(i == 0)(lambda: attention_fwd(True))
            pl.when(i > 0)(lambda: attention_fwd(False))

        @pl.when(i == 0)
        def _wait_rest_of_weights():
            with jax.named_scope('waitw'):
                for c in w_in[1:]:
                    c.wait()

        with jax.named_scope('wo'):
            o = jnp.concatenate([otbuf[g].T for g in range(n_grp)], axis=1)
            ob = o.astype(BF16)
            h = x + _dot(ob, wo_ref[...])
            y2, rstd2 = _ln_stats(h)
            y2b = y2.astype(BF16)
            y2buf[...] = y2b
            y2tbuf[...] = y2.T.astype(BF16)
            yacc[...] = h

        def glu_chunk(c, carry):
            r = pl.multiple_of(c * 128, 128)
            wg_c = wgt_ref[pl.ds(r, 128), :]
            wu_c = wut_ref[pl.ds(r, 128), :]
            wd_c = wd_ref[pl.ds(r, 128), :]
            gate = _dot_nt(y2buf[...], wg_c)
            up = _dot_nt(y2buf[...], wu_c)
            sg = jax.nn.sigmoid(gate)
            hh = (sg * up).astype(BF16)
            yacc[...] += _dot(hh, wd_c)
            dhh = _dot_nt(go_ref[...], wd_c)
            a_wdt[c] += _dot(dytbuf[...], hh)
            du = dhh * sg
            dg = du * up * (1.0 - sg)
            dub = du.astype(BF16)
            dgb = dg.astype(BF16)
            a_wg[c] += _dot(y2tbuf[...], dgb)
            a_wu[c] += _dot(y2tbuf[...], dub)
            dy2acc[...] += _dot(dgb, wg_c) + _dot(dub, wu_c)
            return carry

        with jax.named_scope('glu'):
            lax.fori_loop(0, n_fc, glu_chunk, 0)

        with jax.named_scope('dwo'):
            out_ref[...] = yacc[...].astype(out_ref.dtype)
            dh = go_ref[...].astype(F32) + _ln_bwd(dy2acc[...], y2, rstd2)
            dhbuf[slot] = dh
            dhb = dh.astype(BF16)
            obt = jnp.concatenate([otbuf[g] for g in range(n_grp)], axis=0)
            a_wo[...] += _dot(obt.astype(BF16), dhb)
            do = _dot_nt(dhb, wo_ref[...])
            for g in range(n_grp):
                dotbuf[g] = do[:, g * 128:(g + 1) * 128].T

        @pl.when(i == n_blocks - 1)
        def _flush_mlp_weight_grads():
            with jax.named_scope('flush'):
                s_wo[...] = a_wo[...].astype(BF16)
                for c in range(n_fc):
                    n = min(128, d_ff - c * 128)
                    s_wgt[c * 128:c * 128 + n, :] = a_wg[c].T[:n].astype(BF16)
                    s_wut[c * 128:c * 128 + n, :] = a_wu[c].T[:n].astype(BF16)
                    s_wd[c * 128:c * 128 + n, :] = a_wdt[c].T[:n].astype(BF16)
                for c in w_out[1:]:
                    c.start()

        def dprobs(qb, g, nkt):
            n = nkt(qb) * 128
            q0 = pl.multiple_of(r0 + qb * QB + KW - n, QB)
            cols = slice(qb * QB, (qb + 1) * QB)
            doms = []
            for h in range(HG):
                rows = slice(h * DH, (h + 1) * DH)
                dot_h = dotbuf[g, rows, cols] * linv[qb, g, h]
                dbuf[qb, h] = jnp.sum(dot_h * otbuf[g, rows, cols], axis=0, keepdims=True)
                dot_hb = dot_h.astype(BF16)
                dosb[qb, rows, :] = dot_hb
                zeros = jnp.zeros((DH, QB), BF16)
                doms.append(
                    jnp.concatenate([zeros] * h + [dot_hb] + [zeros] * (HG - 1 - h), axis=0)
                )
            sbuf[qb, 0:n, :] = _dot(vbuf[g, pl.ds(q0, n), :], jnp.concatenate(doms, axis=1))

        def dscores(qb, g, nkt):
            n = nkt(qb) * 128
            old = n - QB
            q0 = pl.multiple_of(r0 + qb * QB + KW - n, QB)
            qn = pl.multiple_of(q0 + old, QB)
            cols = slice(qb * QB, (qb + 1) * QB)
            for h in range(HG):
                rows = slice(h * DH, (h + 1) * DH)
                pb = pbuf[qb, g, h, 0:n, :]
                dpt = sbuf[qb, 0:n, h * QB:(h + 1) * QB]
                dsbuf[h, 0:n, :] = (pb.astype(F32) * (dpt - dbuf[qb, h])).astype(BF16)
                dk = _dot_nt(qtbuf[g, rows, cols], dsbuf[h, 0:n, :])
                dv = _dot_nt(dosb[qb, rows, :], pbuf[qb, g, h, 0:n, :])
                if old:
                    dk_acc[g, rows, pl.ds(q0, old)] += dk[:, :old]
                    dv_acc[g, rows, pl.ds(q0, old)] += dv[:, :old]
                dk_acc[g, rows, pl.ds(qn, QB)] = dk[:, old:]
                dv_acc[g, rows, pl.ds(qn, QB)] = dv[:, old:]
                dqtbuf[slot, g, rows, cols] = _dot(
                    ktbuf[g, rows, pl.ds(q0, n)], dsbuf[h, 0:n, :]
                ) * (DH ** -0.5)

        def attention_bwd(first):
            nkt = nkt_of(first)

            def body(g, carry):
                for qb in range(NQB):
                    if qb + 1 < NQB:
                        dprobs(qb + 1, g, nkt)
                    else:
                        dprobs(0, jnp.minimum(g + 1, n_grp - 1), nkt)
                    dscores(qb, g, nkt)
                return carry

            dprobs(0, 0, nkt)
            lax.fori_loop(0, n_grp, body, 0)

        with jax.named_scope('attn_bwd'):
            pl.when(i == 0)(lambda: attention_bwd(True))
            pl.when(i > 0)(lambda: attention_bwd(False))

    @pl.when(i > 0)
    def _lagged_backward():
        with jax.named_scope('lag'):
            prev = 1 - slot
            y1 = y1buf[prev]
            kv1 = pl.multiple_of((i - 1) * T + W, 128)
            dqkv = jnp.concatenate(
                [dqtbuf[prev, g].T for g in range(n_grp)]
                + [dk_acc[g, :, pl.ds(kv1, T)].T * LN2 for g in range(n_grp)]
                + [dv_acc[g, :, pl.ds(kv1, T)].T for g in range(n_grp)],
                axis=1,
            ).astype(BF16)
            a_wqkv[...] += _dot_tn(y1.astype(BF16), dqkv)
            dy1 = _dot_nt(dqkv, wqkv_ref[...])
            dx_ref[...] = (dhbuf[prev] + _ln_bwd(dy1, y1, r1buf[prev])).astype(dx_ref.dtype)

    @pl.when(i == n_blocks)
    def _finalize():
        with jax.named_scope('final'):
            s_wqkv[...] = a_wqkv[...].astype(BF16)
            w_out[0].start()
            for c in w_out:
                c.wait()


@jax.jit
def pallas_sequential_preLN__sliding_block__glu_gated_glu__prompt_kernel(
    A_x: jax.Array,
    A_wqkv: jax.Array,
    A_wo: jax.Array,
    B_x: jax.Array,
    B_w_gate: jax.Array,
    B_w_up: jax.Array,
    B_w_down: jax.Array,
    grad_out: jax.Array,
):
    del B_x
    B, S, D = A_x.shape
    assert B == 1 and S % T == 0 and T >= W and D % 128 == 0 and D // DH == H
    F = B_w_gate.shape[1]
    x = A_x.reshape(S, D)
    go = grad_out.reshape(S, D)
    nb = S // T
    ng = D // 128
    SP = S + W

    rows_cur = pl.BlockSpec((T, D), lambda i: (jnp.minimum(i, nb - 1), 0))
    rows_prev = pl.BlockSpec((T, D), lambda i: (jnp.maximum(i - 1, 0), 0))
    hbm = pl.BlockSpec(memory_space=pl.ANY)

    in_specs = [rows_cur, rows_cur, hbm, hbm, hbm, hbm, hbm]
    out_specs = [rows_cur, rows_prev, hbm, hbm, hbm, hbm, hbm]
    w_shapes = [(D, 3 * D), (D, D), (F, D), (F, D), (F, D)]
    out_shape = [
        jax.ShapeDtypeStruct((S, D), BF16),
        jax.ShapeDtypeStruct((S, D), BF16),
    ] + [jax.ShapeDtypeStruct(s, BF16) for s in w_shapes]
    FP = pl.cdiv(F, 128) * 128
    scratch = (
        [pltpu.VMEM(s, BF16) for s in [(D, 3 * D), (D, D), (FP, D), (FP, D), (FP, D)]]
        + [pltpu.SemaphoreType.DMA((5,))]
        + [pltpu.VMEM(s, BF16) for s in w_shapes]
        + [pltpu.SemaphoreType.DMA((5,))]
        + [
            pltpu.VMEM((ng, 128, T), BF16),
            pltpu.VMEM((ng, SP, 128), BF16),
            pltpu.VMEM((ng, SP, 128), BF16),
            pltpu.VMEM((ng, 128, SP), BF16),
            pltpu.VMEM((ng, HG, VR, SP), BF16),
            pltpu.VMEM((NQB, ng, HG, KW, QB), BF16),
            pltpu.VMEM((HG, KW, QB), BF16),
            pltpu.VMEM((NQB, KW, HG * QB), F32),
            pltpu.VMEM((NQB, HG, 1, QB), F32),
            pltpu.VMEM((NQB, HG, 1, QB), F32),
            pltpu.VMEM((NQB, 128, QB), BF16),
            pltpu.VMEM((NQB, KW, QB), F32),
            pltpu.VMEM((NQB, ng, HG, 1, QB), F32),
            pltpu.VMEM((ng, 128, T), F32),
            pltpu.VMEM((ng, 128, T), F32),
            pltpu.VMEM((2, ng, 128, T), F32),
            pltpu.VMEM((ng, 128, SP), F32),
            pltpu.VMEM((ng, 128, SP), F32),
            pltpu.VMEM((2, T, D), F32),
            pltpu.VMEM((2, T, D), F32),
            pltpu.VMEM((2, T, 1), F32),
            pltpu.VMEM((D, 3 * D), F32),
            pltpu.VMEM((D, D), F32),
            pltpu.VMEM((FP // 128, D, 128), F32),
            pltpu.VMEM((FP // 128, D, 128), F32),
            pltpu.VMEM((FP // 128, D, 128), F32),
            pltpu.VMEM((T, D), BF16),
            pltpu.VMEM((D, T), BF16),
            pltpu.VMEM((D, T), BF16),
            pltpu.VMEM((T, D), F32),
            pltpu.VMEM((T, D), F32),
        ]
    )
    outs = pl.pallas_call(
        functools.partial(_kernel, n_blocks=nb, d_model=D, d_ff=F),
        grid=(nb + 1,),
        in_specs=in_specs,
        out_specs=out_specs,
        out_shape=out_shape,
        scratch_shapes=scratch,
        compiler_params=pltpu.CompilerParams(
            dimension_semantics=("arbitrary",),
            vmem_limit_bytes=100 * 1024 * 1024,
        ),
    )(x, go, A_wqkv, A_wo, B_w_gate.T, B_w_up.T, B_w_down)
    out, dx = outs[0].reshape(B, S, D), outs[1].reshape(B, S, D)
    return (out, dx, outs[2], outs[3], outs[4].T, outs[5].T, outs[6])
```
